```python
import os as _os
_os.environ.setdefault("JAX_PLATFORMS", "cpu")
import jax
import jax.numpy as jnp

def _softmax(x, axis=-1):
    return jax.nn.softmax(x, axis=axis)
def _gelu(x):
    return jax.nn.gelu(x, approximate=True)
def _silu(x):
    return jax.nn.silu(x)
def _sigmoid(x):
    return jax.nn.sigmoid(x)
def _layernorm(x, axis=-1, eps=1e-5):
    m = jnp.mean(x, axis=axis, keepdims=True)
    v = jnp.var(x, axis=axis, keepdims=True)
    return (x - m) / jnp.sqrt(v + eps)
def _scatter_add(tgt, idx, src, axis=0):
    return tgt.at[idx].add(src)
def _segment_sum(src, seg, n):
    return jax.ops.segment_sum(src, seg, n)
class _Rng:
    def __init__(self, key):
        self._k = key
    def _next(self):
        self._k, sub = jax.random.split(self._k)
        return sub
    def normal(self, shape):
        return jax.random.normal(self._next(), shape, dtype=jnp.bfloat16)
    def randint(self, lo, hi, shape):
        return jax.random.randint(self._next(), shape, lo, hi, dtype=jnp.int32)
    def uniform(self, shape, lo=0.0, hi=1.0):
        return jax.random.uniform(self._next(), shape, jnp.bfloat16, lo, hi)
    def permutation(self, n):
        return jax.random.permutation(self._next(), n)


kernel_name = 'interleave_layers__sliding_local_dilated__glu_gated_reglu__prompt'

def setup_inputs():
    _rng = _Rng(jax.random.key(int.from_bytes(__import__("os").urandom(4), "little")))
    _w = (lambda a: (lambda t: t.astype(jnp.bfloat16) if jnp.issubdtype(t.dtype, jnp.floating) else t)(jnp.asarray(a)))
    def _A_setup():
        B, S, D = 1, 2048, 512
        return {
            "x": _w((lambda *s: _rng.normal(s) * 0.05)(B, S, D)),
            "wqkv": _w((lambda *s: _rng.normal(s) * 0.05)(D, 3 * D)),
            "wo": _w((lambda *s: _rng.normal(s) * 0.05)(D, D)),
        }
    _A_in = _A_setup()

    def _B_setup():
        B, S, D, F = 1, 2048, 512, 1792
        return {
            "x": _w((lambda *s: _rng.normal(s) * 0.05)(B, S, D)),
            "W_gate": _w((lambda *s: _rng.normal(s) * 0.8)(D, F) * (2.0 / D) ** 0.5),
            "W_up": _w((lambda *s: _rng.normal(s) * 0.8)(D, F) * (2.0 / D) ** 0.5),
            "W_down": _w((lambda *s: _rng.normal(s) * 0.8)(F, D) * (1.0 / F) ** 0.5),
        }
    _B_in = _B_setup()

    return {
        "A_x": _A_in["x"],
        "A_wqkv": _A_in["wqkv"],
        "A_wo": _A_in["wo"],
        "B_x": _B_in["x"],
        "B_W_gate": _B_in["W_gate"],
        "B_W_up": _B_in["W_up"],
        "B_W_down": _B_in["W_down"],
    }

def reference(A_x, A_wqkv, A_wo, B_x, B_W_gate, B_W_up, B_W_down):
    def _A_ref(x, wqkv, wo):
        B, S, D = x.shape
        H = 32; Dh = D // H
        W, dil = 8, 2
        qkv = (lambda x, *d: x.transpose(*d))((x @ wqkv).reshape(B, S, 3, H, Dh), 2, 0, 3, 1, 4)
        q, k, v = qkv[0], qkv[1], qkv[2]
        scale = Dh ** -0.5
        pos = jnp.arange(S)
        off = jnp.arange(W) * dil
        idx = pos[:, None] - off[None, :]
        mask = idx >= 0
        idx_c = jnp.where(mask, idx, 0).reshape(-1)
        kg = k[:, :, idx_c, :].reshape(B, H, S, W, Dh)
        vg = v[:, :, idx_c, :].reshape(B, H, S, W, Dh)
        logits = jnp.einsum("bhsd,bhswd->bhsw", q, kg) * scale
        logits = jnp.where(mask[None, None, :, :], logits, -1e9)
        attn = _softmax(logits, axis=-1)
        o = jnp.einsum("bhsw,bhswd->bhsd", attn, vg)
        return (lambda x, *d: x.transpose(*d))(o, 0, 2, 1, 3).reshape(B, S, D) @ wo

    def _B_ref(x, W_gate, W_up, W_down):
        gate = jnp.einsum("bsd,df->bsf", x, W_gate)
        up = jnp.einsum("bsd,df->bsf", x, W_up)
        gate = gate * (lambda x, dt: x.astype(dt))(gate > 0, gate.dtype)
        h = gate * up
        return jnp.einsum("bsf,fd->bsd", h, W_down)

    x = A_x
    x = x + _A_ref(_layernorm(x, axis=-1), A_wqkv, A_wo)
    x = x + _B_ref(_layernorm(x, axis=-1), B_W_gate, B_W_up, B_W_down)
    x = x + _A_ref(_layernorm(x, axis=-1), A_wqkv, A_wo)
    x = x + _B_ref(_layernorm(x, axis=-1), B_W_gate, B_W_up, B_W_down)
    return x
```

```python
import bisect
import functools
import heapq

import jax
import jax.numpy as jnp
from jax import lax
import jax.experimental.pallas as pl
import jax.experimental.pallas.tpu as pltpu

F32, BF16, U32 = jnp.float32, jnp.bfloat16, jnp.uint32
S, D, F = 2048, 512, 1792
WIN = 8
HALO = WIN - 1
NB = 8
EXP_SCALE = 0.25 * 1.4426950408889634
MASKED = -4e9
MXU_LATENCY = 131

LHS7 = ((0, 1, 3), (2, 1, 3), (0, 0, 0), (3, 0, 0), (0, 1, 1), (2, -1, 0), (1, -1, 3))
RHS7 = ((0, 1, 3), (0, 0, 0), (1, -1, 3), (2, -1, 0), (3, 0, 0), (0, 1, 1), (2, 1, 3))
ROWS = (0, 3, 2, 6, 4, 5, 1)
STREAM = (0, 1, 2, 5, 3, 4, 6)


def _pack(x):
    return pltpu.bitcast(x.astype(BF16), U32)


def _unpack(x):
    return pltpu.bitcast(x, BF16)


def _same(x):
    return x


def _mix(recipe, block, gate=_same):
    i, sign, j = recipe
    a = gate(block(i))
    return a if sign == 0 else a + block(j) if sign > 0 else a - block(j)


def _mix7(recipes, blocks):
    return [_mix(r, blocks.__getitem__) for r in recipes]


GMODE = [2]


def _mix_inner(recipes, p, block, gate=_same):
    return _mix7(recipes, [_mix(recipes[p], lambda i: block(2 * (i // 2) + r, 2 * (i % 2) + c),
                                gate if (r == c and GMODE[0] > 0) or (GMODE[0] == 2) or (GMODE[0] == 3 and recipes[p][1]) else _same)
                           for r in range(2) for c in range(2)])


def _add(a, b):
    return [x + y for x, y in zip(a, b)]


def _sub(a, b):
    return [x - y for x, y in zip(a, b)]


def _out4(prod, order, emit=None):
    out = [None] * 4

    def done(i, v):
        out[i] = v
        if emit is not None:
            emit(i, v)

    if order == "stream":
        m1, m2, m3 = prod(0), prod(1), prod(2)
        done(3, _add(_sub(_add(prod(5), m1), m2), m3))
        m4 = prod(3)
        done(2, _add(m2, m4))
        t = _add(m1, m4)
        m5 = prod(4)
        done(1, _add(m3, m5))
        t = _sub(t, m5)
        done(0, _add(t, prod(6)))
    elif order == "rows":
        m1, m4, m3 = prod(0), prod(3), prod(2)
        t = _add(_add(prod(6), m1), m4)
        m5 = prod(4)
        done(0, _sub(t, m5))
        done(1, _add(m3, m5))
        t = _add(_add(prod(5), m1), m3)
        m2 = prod(1)
        done(2, _add(m2, m4))
        done(3, _sub(t, m2))
    else:
        m1 = prod(0) if order >= 1 else None
        u = _add(prod(5), m1) if order >= 2 else m1
        t = _add(prod(6), m1) if order >= 3 else m1
        m2, m4, m3, m5 = prod(1), prod(3), prod(2), prod(4)
        done(2, _add(m2, m4))
        done(1, _add(m3, m5))
        if order == 0:
            t, u = _sub(m4, m5), _sub(m3, m2)
            m1 = prod(0)
            t, u = _add(t, m1), _add(u, m1)
        else:
            t, u = _add(t, _sub(m4, m5)), _add(u, _sub(m3, m2))
        done(3, u if order >= 2 else _add(u, prod(5)))
        done(0, t if order >= 3 else _add(t, prod(6)))
    return out


class _Bank:
    def __init__(self, ref, rows, cols):
        self.ref, self.rows, self.cols = ref, rows, cols
        self.per_row = ref.shape[1] // cols
        self.filled = {}

    def _index(self, n, r0, nr, c0, nc):
        r = (n // self.per_row) * self.rows + r0
        c = (n % self.per_row) * self.cols + c0
        return slice(r, r + nr), slice(c, c + nc)

    def put(self, n, r0, c0, x):
        idx = self._index(n, r0, x.shape[0] // 2, c0, x.shape[1])
        self.ref[idx] = _pack(x)
        for r in range(r0, r0 + x.shape[0] // 2, 8):
            self.filled[n, r] = self.filled.get((n, r), 0) + x.shape[1]
        return idx

    def get(self, n, r0=0, nr=None):
        nr = self.rows if nr is None else nr
        have = {self.filled.get((n, r), 0) for r in range(r0, r0 + nr, 8)}
        assert len(have) == 1 and min(have) > 0 and min(have) % self.cols == 0
        return self.ref[self._index(n, r0, nr, 0, self.cols)]

    def gather(self, idxs):
        acc = functools.reduce(jnp.bitwise_or, [self.ref[idx] for idx in idxs])
        return functools.reduce(jnp.bitwise_or, [
            acc[i:i + 8, j:j + 128]
            for i in range(0, acc.shape[0], 8) for j in range(0, acc.shape[1], 128)])


class _Timeline:
    def __init__(self):
        self.never = self.flag = None
        self.tiles = 0
        self.free = [0] * 4
        self.recent = [[] for _ in range(4)]
        self.syncs = {}
        self.begin = 0
        self.tasks = []
        self.count = 0
        self.now = None
        self.ties = []
        self.times = []
        self.results = []

    def spawn(self, task, at):
        self.count += 1
        heapq.heappush(self.tasks, (at, self.count, task))

    def pace(self, tasks, first, last):
        base = sum(self.free) / 4
        for i, task in enumerate(tasks):
            self.spawn(task, base + first + (last - first) * i / max(len(tasks) - 1, 1))

    def run(self, until=float("inf")):
        while self.tasks and self.tasks[0][0] <= until:
            self.now, _, task = heapq.heappop(self.tasks)
            sleep = next(task, None)
            if sleep is not None:
                self.spawn(task, self.now + sleep)
        self.now = None

    def token(self):
        i = bisect.bisect_right(self.times, self.now)
        if i == 0:
            return None
        m, r = self.results[i - 1]
        return m[r:r + 8, :128]

    def select(self, reg, x):
        if reg.dtype != x.dtype:
            reg = pltpu.bitcast(reg, x.dtype)
        reps = (x.shape[0] // 8, x.shape[1] // 128)
        if reps == (1, 1):
            return jnp.where(self.never, reg, x)
        return jnp.where(jnp.tile(self.flag, reps) != 0, jnp.tile(reg, reps), x)

    def gate(self, x):
        token = self.token()
        return x if token is None else self.select(token, x)

    def rows(self):
        token = self.token()
        if token is None:
            return pl.ds
        zero = jnp.where(self.never, pltpu.bitcast(token, jnp.int32), 0)[0, 0]
        return lambda start, size: pl.ds(pl.multiple_of(zero + start, 16), size)

    def tie(self, x, after):
        self.ties.append((self.now + after, x if x.dtype == U32 else pltpu.bitcast(x, U32)))

    def lockstep(self, at):
        if at not in self.syncs:
            picks = {}
            for recent in self.recent:
                for begin, n, m, col in reversed(recent):
                    r = min((at - 10 - MXU_LATENCY - begin) // 8 * 8, m.shape[0] - 8)
                    if r >= 0:
                        picks[n, r, col] = m
                        break
            regs = [pltpu.bitcast(m[r:r + 8, col:col + 128], U32) for (_, r, col), m in picks.items()]
            self.syncs[at] = functools.reduce(jnp.bitwise_or, regs) if regs else None
        return self.syncs[at]

    def dot(self, lhs, rhs, nt=False):
        self.run(max(self.times[-1:] + [min(self.free)]))
        lhs, rhs = lhs(), rhs()
        rhs = rhs if rhs.dtype == BF16 else _unpack(rhs)
        nreg, kt = lhs.shape[0] // 8, lhs.shape[1] // 128
        tiles = kt * (rhs.shape[0 if nt else 1] // 128)
        slots = [(self.tiles + i) % 4 for i in range(tiles)]
        starts = [self.free[i] for i in slots]
        self.begin = max(starts)
        ties, later = {}, []
        for t, x in self.ties:
            reg = max(int((t - self.begin) // 16), 0)
            if reg >= nreg:
                later.append((t, x))
            else:
                ties[reg] = x if reg not in ties else ties[reg] | x
        self.ties = later
        sync = self.lockstep(min(starts))
        if sync is not None:
            ties[0] = sync if 0 not in ties else ties[0] | sync
        parts, r = [], 0
        for reg in sorted(ties):
            if 8 * reg > r:
                parts.append(lhs[r:8 * reg])
            row = lhs[8 * reg:8 * reg + 8]
            if reg == 0 or kt == 1:
                parts.append(self.select(ties[reg], row))
            else:
                parts.append(jnp.concatenate([self.select(ties[reg], row[:, :128]), row[:, 128:]], axis=1))
            r = 8 * reg + 8
        if r < lhs.shape[0]:
            parts.append(lhs[r:])
        lhs = jnp.concatenate(parts, axis=0)
        dims = (((1,), (1 if nt else 0,)), ((), ()))
        m = lax.dot_general(_unpack(lhs), rhs, dims, preferred_element_type=F32)
        for n, i in enumerate(slots):
            self.recent[i] = self.recent[i][-2:] + [(self.free[i], self.tiles, m, 128 * (n // kt))]
            self.free[i] += 16 * nreg
        for r in range(0, 16 * nreg, 8):
            t = starts[0] + MXU_LATENCY + r
            i = bisect.bisect_right(self.times, t)
            self.times.insert(i, t)
            self.results.insert(i, (m, r))
        self.tiles += tiles
        return m

    def out16(self, prod, order, emit=None):
        def outer(p):
            return [b[0] for b in _out4(lambda q: [prod(7 * p + q)], -self.tiles % 4)]

        def leave(i, v):
            for j in (2, 1, 3, 0):
                emit(2 * (i // 2) + j // 2, 2 * (i % 2) + j % 2, v[j])

        return _out4(outer, order, None if emit is None else leave)


def _kernel(x_hbm, wqkv_hbm, wo_hbm, wg_hbm, wu_hbm, wd_hbm, out_hbm,
            x_in, wqkv_in, wo_in, wg_in, wu_in, wd_in, out_st,
            x_w, wo_w, out_w, pack_r, xs, qs, ks, vs, os_,
            eye_r, wqt_r, xb7_r, wq7_r, oa7_r, wo7_r, xb49_r, wq49_r, oa49_r, wo49_r,
            xa_r, wgu_r, ha49_r, ha7_r, wd49_r, wd7_r,
            sems, *, cfg):
    clock = _Timeline()
    eye, wqt = _Bank(eye_r, 64, 128), _Bank(wqt_r, 192, 128)
    xb7, wq7 = _Bank(xb7_r, 256, 256), _Bank(wq7_r, 96, 256)
    oa7, wo7 = _Bank(oa7_r, 256, 256), _Bank(wo7_r, 128, 256)
    xb49, wq49 = _Bank(xb49_r, 64, 128), _Bank(wq49_r, 96, 128)
    oa49, wo49 = _Bank(oa49_r, 128, 128), _Bank(wo49_r, 64, 128)
    xa, wgu = _Bank(xa_r, 128, 128), _Bank(wgu_r, 64, 128)
    ha49, ha7 = _Bank(ha49_r, 128, 128), _Bank(ha7_r, 256, 128)
    wd49, wd7 = _Bank(wd49_r, 64, 128), _Bank(wd7_r, 64, 128)
    part = functools.partial
    ws = cfg["ws"]
    GMODE[0] = cfg["gmode"]

    def x_part(h, s, m0=0, m=64):
        return x_hbm.at[pl.ds(64 * h + m0, m), pl.ds(8 * s, 8)], x_in.at[h, s, pl.ds(m0, m)]

    def wqkv_part(g, n):
        return [(wqkv_hbm.at[:, pl.ds(c, 128 * n)], wqkv_in.at[:, pl.ds(c, 128 * n)])
                for c in range(128 * g, 3 * D, D)]

    waves = [[pltpu.make_async_copy(src, dst, sems.at[n]) for src, dst in wave] for n, wave in enumerate([
        [x_part(0, 1, 0, 32)],
        wqkv_part(0, 1) + [x_part(0, 1, 32, 32)],
        [x_part(0, 0)] + wqkv_part(1, 1),
        wqkv_part(2, 2) + [x_part(1, 1), x_part(1, 0)],
        [(wo_hbm, wo_in), (wg_hbm, wg_in), (wu_hbm, wu_in), (wd_hbm, wd_in)],
    ])]

    def start(copies):
        for copy in copies:
            copy.start()

    def wait(n):
        with jax.named_scope("wait%d" % n):
            for copy in waves[n]:
                copy.wait()

    def once(fn, *args):
        fn(*args)
        return
        yield

    def put7(bank, n0, r0, c0, values, stride=1):
        idx = [bank.put(n0 + stride * i, r0, c0, v) for i, v in enumerate(values)]
        if len(idx) == 7 and cfg["few"]:
            lhs = bank in (wq49, oa49, xa, ha49)
            idx = [idx[i] for i in cfg["few"][0 if lhs else 1]]
        clock.tie(bank.gather(idx), ws)

    def build7(recipes, p, block, bank, n0, r0, gate=_same, fresh=lambda: None):
        sums, idx = {}, []
        plan = ((0, (2,)), (2, (5,)), (3, (0, 1, 3)), (1, (4, 6))) if recipes is LHS7 else (
            (0, (1,)), (1, (5,)), (3, (0, 2, 4)), (2, (3, 6)))
        at = fresh()
        for j, ready in plan:
            sums[j] = _mix(recipes[p],
                           lambda i: block(2 * (i // 2) + j // 2, 2 * (i % 2) + j % 2, *([at] if at else [])),
                           gate if recipes[p][1] or j in (0, 3) else _same)
            idx += [bank.put(n0 + q, r0, 0, _mix(recipes[q], sums.__getitem__)) for q in ready]
            if j != plan[-1][0]:
                yield cfg["bstep"]
        clock.tie(bank.gather(idx), cfg["wb"])

    def layernorm(load, n):
        x, mean, c, var = [], [], [], []
        for i in range(n):
            x.append(load(i))
            s = ((clock.gate(x[i][:, :128]) + x[i][:, 128:256]) + x[i][:, 256:384]) + x[i][:, 384:]
            mean.append(jnp.sum(s, axis=-1, keepdims=True) * (1.0 / D))
            yield cfg["ln_step"]
        yield cfg["ln_wait"] - n * cfg["ln_step"]
        for i in range(n):
            c.append(x[i] - mean[i])
            var.append(jnp.sum(c[i] * c[i], axis=-1, keepdims=True) * (1.0 / D))
            yield cfg["ln_step"]
        yield cfg["ln_wait"] - n * cfg["ln_step"] + 30
        if cfg["again"]:
            c = [x[i] - jnp.tile(clock.gate(jnp.broadcast_to(mean[i], (8, 128))), (1, 4)) for i in range(n)]
        y = [c[i] * (jnp.exp2(jnp.log(var[i] + 1e-5) * (-0.5 * 1.4426950408889634)) if cfg["elog"] else lax.rsqrt(var[i] + 1e-5)) for i in range(n)]
        if n == 8:
            bits = functools.reduce(jnp.bitwise_or, [pltpu.bitcast(v[:, 384:], U32) for v in y])
            clock.tie(bits, ws)
        else:
            yield n * cfg["ln_step"]
        return [jnp.concatenate(y[i:i + 2], axis=0) for i in range(0, n, 2)]

    def norm49(pieces, recipes, bank, order):
        done = {}

        def norm(i, rows):
            done[i] = yield from layernorm(lambda n: xs[pl.ds(rows[n // 2] + 8 * (n % 2), 8), :], 8)

        def step(p, i, n0, r0):
            tile = lambda token, k: done[i][token][:, 128 * k:128 * k + 128]
            return build7(recipes, p, tile if recipes is LHS7 else lambda k, token: tile(token, k),
                          bank, n0 + 7 * p, r0, clock.gate)

        return ([norm(i, rows) for i, (rows, _, _) in enumerate(pieces)],
                [step(p, i, n0, r0) for p in order for i, (_, n0, r0) in enumerate(pieces)])

    def prep_qkv7(g):
        def slab(k):
            w = jnp.concatenate([
                clock.dot(part(eye.get, 0), lambda: wqkv_in[128 * k:128 * k + 128, c0:c0 + 128], nt=True)
                for c0 in range(128 * g, 3 * D, D)], axis=0)
            wqt.put(4 * g + k, 0, 0, w)
            return w
        for kt in range(2):
            lo, hi = slab(kt), slab(2 + kt)
            for p, w in enumerate(_mix7(LHS7, (lo[:192], hi[:192], lo[192:], hi[192:]))):
                wq7.put(7 * g + p, 0, 128 * kt, w)

    def prep_qkv49(r):
        def step(p, u):
            return build7(LHS7, p, lambda b, k: _unpack(clock.gate(
                wqt.get(4 * (2 * r + b // 2) + k, 96 * (b % 2) + 8 * u, 8))).astype(F32),
                wq49, 49 * r + 7 * p, 8 * u)
        return [step(p, u) for p in STREAM for u in range(12)]

    def wo_rows(g, t, dd):
        w = clock.gate(wo_w[t, pl.ds(64 * g + dd, 8, stride=8), :])
        return jnp.concatenate([pltpu.bitcast(w << 16, F32),
                                pltpu.bitcast(w & jnp.uint32(0xFFFF0000), F32)], axis=0)

    def prep_wo7():
        def step(gi, ti, dd):
            put7(wo7, 0, 64 * gi + 8 * dd, 128 * ti,
                 _mix7(RHS7, [wo_rows(g, t, dd) for g in (gi, 2 + gi) for t in (ti, 2 + ti)]))
        return [once(step, gi, ti, dd) for gi in range(2) for ti in range(2) for dd in range(8)]

    def prep_wo49():
        def step(p, dd):
            return build7(RHS7, p, lambda g, t: wo_rows(g, t, dd), wo49, 7 * p, 8 * dd)
        return [step(p, dd) for p in STREAM for dd in range(8)]

    slabs = {}

    def slab(name, ref, row, col):
        if (name, row, col) not in slabs:
            slabs[name, row, col] = pltpu.bitcast(ref[row:row + 16, col:col + 128], U32)
        return _unpack(clock.gate(slabs[name, row, col])).astype(F32)

    def prep_gu(j):
        def block(u, k, n):
            return slab(n // 2, (wg_in, wu_in)[n // 2], 128 * k + 16 * u, 896 * (n % 2) + 128 * j)
        return [build7(RHS7, p, part(block, u), wgu, 49 * j + 7 * p, 8 * u) for p in ROWS for u in range(8)]

    def prep_down():
        def block(jj, u, k, n):
            return slab(2, wd_in, 128 * (7 * (k // 2) + 2 * jj + k % 2) + 16 * u, 128 * n)

        def odd(u, ti):
            put7(wd7, ti, 8 * u, 0, _mix7(RHS7, [slab(2, wd_in, 128 * ft + 16 * u, 128 * t)
                                                 for ft in (6, 13) for t in (ti, 2 + ti)]), stride=2)

        return ([once(odd, u, ti) for u in range(8) for ti in range(2)]
                + [build7(RHS7, p, part(block, jj, u), wd49, 49 * jj + 7 * p, 8 * u)
                   for p in STREAM for jj in range(3) for u in range(8)])

    def token_row(h, q, c):
        return 1024 * h + 256 * q + 32 * c

    def norm_qkv7(h, s, quarters=range(4)):
        def task(pair, q, u):
            m0 = 16 * q + 8 * u
            if pair % 2 == 0:
                for t in range(4):
                    x_w[h, s, t, 4 * m0:4 * m0 + 32, :] = pltpu.bitcast(
                        x_in[h, s, m0:m0 + 8, :, 128 * t:128 * t + 128].reshape(64, 128), U32)
            rows = [token_row(h, q, 2 * pair + n) + 16 * u for n in range(2)]
            for n in range(2):
                xs[pl.ds(rows[n], 16), :] = jnp.concatenate(
                    [_unpack(clock.gate(x_w[h, s, t, pl.ds(4 * m0 + 2 * (pair % 2) + n, 8, stride=4), :])
                             ).astype(F32) for t in range(4)], axis=1)
            xn = yield from layernorm(lambda i: xs[pl.ds(rows[i // 2] + 8 * (i % 2), 8), :], 4)
            put7(xb7, 7 * h, 64 * pair + 16 * q + 8 * u, 0,
                 _mix7(RHS7, (xn[0][:, :256], xn[1][:, :256], xn[0][:, 256:], xn[1][:, 256:])))
        return [task(pair, q, u) for q in quarters for u in range(2) for pair in (2 * s, 2 * s + 1)]

    def norm_qkv49(h, s):
        return norm49([([token_row(h, q, 4 * s + n) + 16 * u for n in range(4)], 49 * (2 * h + s), 16 * q + 8 * u)
                       for q in range(4) for u in range(2)], RHS7, xb49, STREAM)

    rolled = {(i, h, g, c): 0 for i in (False, True) for h in range(2) for g in range(4) for c in range(NB)}
    own = lambda c: slice(128 * (HALO + c), 128 * (HALO + c + 1))

    def wrap(ref, h, g, c):
        lane = lax.broadcasted_iota(jnp.int32, (32, 128), 1)
        for r in range(0, 128, 32):
            x = pltpu.roll((clock.gate if cfg["wgate"] else _same)(ref[h, g, r:r + 32, own(c)]), 2, 1)
            if h > 0:
                x = jnp.where(lane < 2, ref[h - 1, g, r:r + 32, own(c - NB)], x)
            ref[h, g, r:r + 32, own(c - NB)] = x
            bits = pltpu.bitcast(x, U32)
            clock.tie((bits[:8] | bits[8:16]) | (bits[16:24] | bits[24:]), cfg["wr"])
            yield 32
        rolled[ref is ks, h, g, c] += 1

    arrived = set()

    def keep_qkv(h, g, c, half, x, delay):
        if half == 0:
            qs[h, g, :, 128 * c:128 * c + 128] = x[:128]
            ks[h, g, :64, own(c)] = x[128:]
        else:
            ks[h, g, 64:, own(c)] = x[:64]
            vs[h, g, :, own(c)] = x[64:]
        arrived.symmetric_difference_update({(h, g, c)})
        if c > 0:
            at = clock.begin + MXU_LATENCY + 140 + delay
            if half == 1:
                clock.spawn(wrap(vs, h, g, c), at)
            if (h, g, c) not in arrived:
                clock.spawn(wrap(ks, h, g, c), at + (64 if half == 1 else 0))

    def qkv7(h, g, sets=(1, 0)):
        for s in sets:
            def emit(i, v):
                for n in range(2):
                    keep_qkv(h, g, 4 * s + 2 * n + i % 2, i // 2, v[0][:, 128 * n:128 * n + 128], 96 * (1 - n))
            _out4(lambda p: [clock.dot(part(wq7.get, 7 * g + p), part(xb7.get, 7 * h + p, 128 * s, 128), nt=True)],
                  "stream", emit)

    def qkv49(h, r, s):
        clock.out16(lambda p: clock.dot(part(wq49.get, 49 * r + p), part(xb49.get, 49 * (2 * h + s) + p), nt=True),
                 "stream", lambda b, n, x: keep_qkv(h, 2 * r + b // 2, 4 * s + n, b % 2, x, 90 * (2 * (b % 2) + n % 2)))

    attended = {}

    def attend(h, layer, g, c):
        step = cfg["astep"]
        lane = lax.broadcasted_iota(jnp.int32, (8, 128), 1)
        assert all(rolled[i, h, g, n] == layer + 1
                   for i in (False, True) for n in {1} | set(range(c + 1, NB))), (h, g, c, clock.now, clock.free)
        logit = [None] * WIN
        for d in range(16):
            q = clock.gate(qs[h, g, 8 * d:8 * d + 8, 128 * c:128 * c + 128])
            k = ks[h, g, 8 * d:8 * d + 8, 128 * c:128 * (c + WIN)]
            for w in range(WIN):
                t = q * k[:, 128 * (HALO - w):128 * (WIN - w)]
                logit[w] = t if d == 0 else logit[w] + t
            yield step
        if h == 0:
            for w in range(c + 1, WIN):
                logit[w] = jnp.where(lane < 2, MASKED, logit[w])
        top = functools.reduce(jnp.maximum, logit)
        e = [jnp.exp2((l - top) * EXP_SCALE) for l in logit]
        inv = 1.0 / functools.reduce(jnp.add, e)
        prob = [x * inv for x in e]
        yield cfg["agap"]
        ns = cfg["pv"]
        o = [None] * ns
        order = [(w, i) for w in range(WIN) for i in range(ns)]
        for w, i in (order if cfg["pvw"] else sorted(order, key=lambda x: x[::-1])):
            t = jnp.tile(clock.gate(prob[w]), (16 // ns, 1)) * vs[h, g, 128 // ns * i:128 // ns * (i + 1), own(c - w)]
            o[i] = t if w == 0 else o[i] + t
            yield 2 * step / ns
        o = jnp.concatenate(o, axis=0).T
        os_[h, g, c] = o
        attended[h, g, c] = layer
        clock.tie(o[120:], cfg["wt"])
        if layer == 0:
            yield cfg["wt"]
            for p in (((2, 5), ()), ((0, 4, 6), (1, 3)))[g // 2][c % 2]:
                for r in (0, 64):
                    v = _mix(LHS7[p], lambda i: os_[h, g % 2 + 2 * (i % 2), c // 2 * 2 + i // 2, r:r + 64],
                             clock.gate)
                    put7(oa7, 7 * h + p, 64 * (c // 2) + r // 2, 128 * (g % 2), [v])
                    yield 30

    def heads49(layer, h, s, _):
        def block(r, n, g):
            assert attended[h, g, 4 * s + n] == layer
            return os_[h, g, 4 * s + n, r:r + 16]

        def step(p, r):
            return build7(LHS7, p, part(block, r), oa49, 7 * p, 64 * s + r // 2, clock.gate)
        return [step(p, r) for p in STREAM for r in range(0, 128, 16)]

    def add_tokens(h, c, cols, x):
        for q in range(4):
            r = pl.ds(token_row(h, q, c), 32)
            xs[r, cols] = xs[r, cols] + x[32 * q:32 * q + 32]

    def out_proj7(h):
        def emit(i, v):
            for pair in range(4):
                add_tokens(h, 2 * pair + i // 2, pl.ds(256 * (i % 2), 256), v[0][128 * pair:128 * pair + 128])
        _out4(lambda p: [clock.dot(part(oa7.get, 7 * h + p), part(wo7.get, p))], "stream", emit)

    def out_proj49(h):
        def emit(n, t, x):
            for s in range(2):
                add_tokens(h, 4 * s + n, pl.ds(128 * t, 128), x[128 * s:128 * s + 128])
        clock.out16(lambda p: clock.dot(part(oa49.get, p), part(wo49.get, p)), "stream", emit)

    def norm_ffn(h, length, split):
        norms, steps = norm49([([token_row(h, q, 0) + 16 * u for q in range(4)], 49 * h, 8 * u)
                               for u in range(16)], LHS7, xa, ROWS)
        return [(norms, cfg["lead"], split * length - cfg["ll"]), (steps, split * length, length + cfg["jit"])]

    def gate_up(h, groups=range(4)):
        def tile(j):
            g1, u1, g2, u2 = clock.out16(lambda p: clock.dot(part(xa.get, 49 * h + p), part(wgu.get, 49 * j + p)), "rows")
            hid = [jnp.maximum(g, 0.0) * u for g, u in zip(g1 + g2, u1 + u2)]
            return [hid[2 * q:2 * q + 2] for q in range(4)]

        def hidden49(jj, pair, p, r):
            return build7(LHS7, p, lambda q, k: pair[k % 2][q][k // 2][r:r + 16],
                          ha49, 49 * jj + 7 * p, r // 2, clock.gate)

        def hidden7(a, p, ri, r):
            put7(ha7, p, 128 * ri + r // 2, 0,
                 [_mix(LHS7[p], lambda i: a[2 * (i // 2) + ri][i % 2][r:r + 64], clock.gate)])

        for jj in groups:
            if jj == 3:
                a = tile(6)
                clock.pace([once(hidden7, a, p, ri, r) for p in STREAM for ri in range(2) for r in range(0, 256, 64)],
                        MXU_LATENCY + 200, cfg["h7"])
                break
            pair = tile(2 * jj), tile(2 * jj + 1)
            if jj < 2:
                skip = cfg["skip"] if len(groups) == 1 else 0
                clock.pace([hidden49(jj, pair, p, r) for r in range(0, 256, 16) for p in range(7)],
                        skip + MXU_LATENCY, skip + 2 * 3136)
            else:
                clock.pace([hidden49(jj, pair, p, r) for p in STREAM for r in range(0, 256, 16)],
                        MXU_LATENCY + 200, cfg["h49"])

    out_dmas = []

    def finish(h, q, t, y, step):
        for c in range(NB):
            idx = slice(16 * c, 16 * c + 16), slice(128 * t, 128 * t + 128)
            pack_r[idx] = _pack((clock.gate if step else _same)(y[32 * c:32 * c + 32]))
            out_w[h, t, pl.ds(128 * q + c, 16, stride=8), :] = pack_r[idx]
            yield step
        out_st[pl.ds(token_row(h, q, 0), 256), pl.ds(128 * t, 128)] = _unpack(out_w[h, t, 128 * q:128 * q + 128, :])

    def send(row, rows, col, cols):
        idx = pl.ds(row, rows), pl.ds(col, cols)
        out_dmas.append(pltpu.make_async_copy(out_st.at[idx], out_hbm.at[idx], sems.at[len(waves)]))
        out_dmas[-1].start()

    early = {}

    def down(h, last, only=None):
        def outer(p):
            def inner(q):
                return [functools.reduce(jnp.add, [
                    clock.dot(part(ha49.get, 49 * jj + 7 * p + q), part(wd49.get, 49 * jj + 7 * p + q))
                    for jj in range(3)])]

            def odd():
                return [clock.dot(part(ha7.get, p, 128 * ri, 128), part(wd7.get, 2 * p + ci))
                        for ri in range(2) for ci in range(2)]

            if p == 6:
                e = odd()
                if last and h == 1:
                    clock.run()
                    send(1024, 512, 256, 256)
                    send(1536, 512, 0, 512)
                return _add(e, [b[0] for b in _out4(inner, "stream")])
            return _add([b[0] for b in _out4(inner, "stream")], odd())

        def emit(i, v):
            for n in (3, 2, 1, 0):
                q, t = 2 * (i // 2) + n // 2, 2 * (i % 2) + n % 2
                idx = (pl.ds(token_row(h, q, 0), 256), pl.ds(128 * t, 128))
                y = xs[idx] + v[n]
                if last:
                    step = 0 if h == 1 and i < 2 else cfg["fstep"]
                    clock.spawn(finish(h, q, t, y, step), clock.begin + MXU_LATENCY + 256 + 8 * step * n)
                else:
                    xs[idx] = y

        if only is not None:
            early.update({p: outer(p) for p in only})
        else:
            _out4(lambda p: early.pop(p) if p in early else outer(p), "stream", emit)

    start(waves[0] + waves[1])
    ri = lax.broadcasted_iota(jnp.int32, (128, 128), 0)
    ci = lax.broadcasted_iota(jnp.int32, (128, 128), 1)
    eye.put(0, 0, 0, jnp.where(ci == (ri & 7) * 16 + (ri >> 3), 1.0, 0.0))
    wait(0)
    start(waves[2])
    clock.never = jnp.abs(x_in[0, 1, 0, :, :128].astype(F32)) < 0.0
    clock.flag = jnp.where(clock.never, 1, 0)
    clock.pace(norm_qkv7(0, 1, (0, 1)), 0, 200)
    clock.run()
    wait(1)
    start(waves[3])
    clock.pace(norm_qkv7(0, 1, (2, 3)), 0, 200)
    clock.run()
    clock.ties = []
    prep_qkv7(0)

    def third_wave():
        wait(4)
        for t in range(4):
            wo_w[t] = pltpu.bitcast(wo_in[:, 128 * t:128 * t + 128], U32)

    Q, O, Q2, O2, G, DN = 2688, 3584, 2352, 3136, 21952, 11200
    lead = cfg["lead"]
    lt = 32 * cfg["astep"] + cfg["agap"] + cfg["wt"]
    la = lt + 180 + ws
    lq = 2 * cfg["ln_wait"] + 30 + 4 * cfg["ln_step"] + ws
    ln = 2 * cfg["ln_wait"] + 30 + 8 * cfg["ln_step"] + 7 * cfg["nstep"] + ws
    ls = ws + 100
    ll = cfg["ll"]
    att0, att1 = [[attend(h, 0, g, c) for g in range(4) for c in reversed(range(NB))] for h in range(2)]
    att2, att3 = [[attend(h, 1, g, 4 * s + c) for r in range(2) for s in (1, 0) for g in (2 * r, 2 * r + 1)
                   for c in reversed(range(4))] for h in range(2)]
    J, P = 3136, 1600
    n1, n2, n3 = cfg["na"]
    m1, m2 = cfg["ma"]
    nd, ng = cfg["nd"], cfg["ng"]
    first, rest = tuple(range(ng)), tuple(range(ng, 4))

    def second_attention(h, att):
        (ln1, st1), (ln0, st0) = norm_qkv49(h, 1), norm_qkv49(h, 0)
        w = 2 * ng * J
        return [
            (part(gate_up, 1 - h, first), [(ln1, lead, 0.25 * w), (st1, 0.25 * w + ll, 0.8 * w),
                                           (ln0, 0.4 * w, 0.8 * w - ll), (st0, 0.8 * w, w + Q2 + 1000)]
             + ([(prep_qkv49(1), 0, w + Q2)] if h == 0 else [])),
            (part(qkv49, h, 0, 1), []),
            (part(qkv49, h, 0, 0), []),
            (part(qkv49, h, 1, 1), [(att[:m1], 800, 2 * Q2 - 300)]),
            (part(qkv49, h, 1, 0), []),
            (part(gate_up, 1 - h, rest), [(att[m1:m1 + m2], 300, G - w - 300)]
             + ([(prep_wo49(), 0, G - w)] if h == 0 else [])),
            (part(down, 1 - h, h == 1, STREAM[:nd]),
             [(att[m1 + m2:], 300, P * nd - lt - 1300), (heads49(1, h, 1, 24), cfg["hs"], P * nd - 1000),
              (heads49(1, h, 0, 32), P * nd - 1200, P * nd + 1500)]),
            (part(out_proj49, h), []),
            (part(down, 1 - h, h == 1), norm_ffn(h, DN - P * nd, cfg["nsplit"])),
        ]

    schedule = [
        (part(qkv7, 0, 0, (1,)), []),
        (lambda: (wait(2), start(waves[4][:2]), prep_qkv7(1)), [(norm_qkv7(0, 0), 150, 384 + Q / 2 - lq + ws - 100)]),
        (part(qkv7, 0, 1, (1,)), []),
        (part(qkv7, 0, 0, (0,)), []),
        (part(qkv7, 0, 1, (0,)), []),
        (lambda: (wait(3), start(waves[4][2:]),
                  prep_qkv7(2), prep_qkv7(3)),
         [(att0[:16], 150, 768 + 2 * Q - 100), (att0[16:], 768 + 2 * Q + 250, 768 + 4.5 * Q - la + 300),
          (norm_qkv7(1, 1) + norm_qkv7(1, 0), lead, 768 + 3 * Q - lq)]),
        (part(qkv7, 0, 2), []),
        (part(qkv7, 0, 3), []),
        (part(qkv7, 1, 0, (1,)), []),
        (part(qkv7, 1, 1, (1,)), []),
        (third_wave, []),
        (part(qkv7, 1, 0, (0,)), [(prep_wo7(), lead, 1.5 * Q - ls)]),
        (part(qkv7, 1, 1, (0,)), []),
        (part(qkv7, 1, 2, (1,)), []),
        (part(out_proj7, 0), [(prep_gu(0) + prep_gu(1), 0, O + cfg["pq"] * Q), (att1[:n1], 400, O - 300)]),
        (part(qkv7, 1, 2, (0,)), norm_ffn(0, 1.5 * Q, cfg["nsplit"])),
        (part(qkv7, 1, 3), []),
        (part(gate_up, 0), [(prep_gu(j), J * (j - 1), J * j - 100) for j in range(2, 7)]
         + [(att1[n1:n1 + n2], J, 2 * J), (att1[n1 + n2:n1 + n2 + n3], 2 * J + 600, G - 300),
            (prep_down(), 6 * J, G + O + cfg["pd"])]),
        (part(down, 0, False, STREAM[:nd]), [(att1[n1 + n2 + n3:], 200, P * nd - la + 300)]),
        (part(out_proj7, 1), []),
        (part(down, 0, False), norm_ffn(1, DN - P * nd, cfg["nsplit"]) + [(prep_qkv49(0), 2000, DN - P * nd + J)]),
        *second_attention(0, att2),
        *second_attention(1, att3),
        (part(gate_up, 1, (0,)), []),
        (part(send, 0, 1024, 0, 512), []),
        (part(gate_up, 1, (1, 2, 3)), []),
        (part(down, 1, True), []),
        (lambda: (clock.run(), send(1024, 512, 0, 256)), []),
    ]
    for n, (phase, side) in enumerate(schedule[:cfg["upto"]]):
        for job in side:
            clock.pace(*job)
        if cfg["scopes"]:
            with jax.named_scope("ph%02d" % n):
                phase()
        else:
            phase()
    if cfg["upto"] < len(schedule):
        while clock.tiles % 4:
            xs[:256, :128] += clock.dot(part(xa.get, 0), part(wgu.get, clock.tiles % 4))
        for h in range(2):
            for q in range(4):
                for t in range(4):
                    list(finish(h, q, t, xs[pl.ds(1024 * h + 256 * q, 256), pl.ds(128 * t, 128)], 0))
        send(0, S, 0, D)
    else:
        assert not clock.tasks
    for d in out_dmas:
        d.wait()


DEFAULT_CFG = dict(lead=200, upto=99, scopes=False, tail=None, early=0, pq=1, pg=0, pd=5000, n1=5, n2=10, n3=25, nd=3, skip=0, fstep=40, bstep=0, wb=400, ll=560, jit=1800, nsplit=0.55, na=(6, 6, 12), ma=(7, 18), ng=1, hs=1400, again=False, pv=1, pvw=False, few=None, gmode=3, wgate=False, elog=True,
                   astep=14, agap=50, wt=350, ws=400, wr=500,
                   ln_step=14, ln_wait=190, nstep=45, h7=5000, h49=4500)


def build(cfg):
    def fn(A_x, A_wqkv, A_wo, B_x, B_W_gate, B_W_up, B_W_down):
        del B_x
        vm = pltpu.VMEM
        scratch = [
            vm((2, 2, 64, 8, D), BF16),
            vm((D, 3 * D), BF16),
            vm((D, D), BF16),
            vm((D, F), BF16),
            vm((D, F), BF16),
            vm((F, D), BF16),
            vm((S, D), BF16),
            vm((2, 2, 4, 256, 128), U32),
            vm((4, 256, 128), U32),
            vm((2, 4, 512, 128), U32),
            vm((128, D), U32),
            vm((S, D), F32),
            vm((2, 4, 128, 128 * NB), F32),
            vm((2, 4, 128, 128 * (NB + HALO)), F32),
            vm((2, 4, 128, 128 * (NB + HALO)), F32),
            vm((2, 4, NB, 128, 128), F32),
            vm((64, 256), U32),
            vm((4 * 192, 512), U32),
            vm((14 * 256, 256), U32),
            vm((28 * 96, 256), U32),
            vm((14 * 256, 256), U32),
            vm((7 * 128, 256), U32),
            vm((28 * 64, 896), U32),
            vm((14 * 96, 896), U32),
            vm((7 * 128, 896), U32),
            vm((7 * 64, 896), U32),
            vm((14 * 128, 896), U32),
            vm((49 * 64, 896), U32),
            vm((21 * 128, 896), U32),
            vm((256, 896), U32),
            vm((21 * 64, 896), U32),
            vm((2 * 64, 896), U32),
            pltpu.SemaphoreType.DMA((6,)),
        ]
        any_spec = pl.BlockSpec(memory_space=pl.ANY)
        out = pl.pallas_call(
            functools.partial(_kernel, cfg=cfg),
            out_shape=jax.ShapeDtypeStruct((S, D), BF16),
            in_specs=[any_spec] * 6,
            out_specs=any_spec,
            scratch_shapes=scratch,
            compiler_params=pltpu.CompilerParams(vmem_limit_bytes=110 * 2**20),
            name="fused",
        )(A_x.reshape(S // 16, 16, D), A_wqkv, A_wo, B_W_gate, B_W_up, B_W_down)
        return out.reshape(1, S, D)
    return fn


_fused = build(DEFAULT_CFG)


@jax.jit
def pallas_interleave_layers__sliding_local_dilated__glu_gated_reglu__prompt_kernel(
    A_x: jax.Array,
    A_wqkv: jax.Array,
    A_wo: jax.Array,
    B_x: jax.Array,
    B_W_gate: jax.Array,
    B_W_up: jax.Array,
    B_W_down: jax.Array,
):
    return _fused(A_x, A_wqkv, A_wo, B_x, B_W_gate, B_W_up, B_W_down)
```

```python
import bisect
import functools
import heapq

import jax
import jax.numpy as jnp
from jax import lax
import jax.experimental.pallas as pl
import jax.experimental.pallas.tpu as pltpu
import numpy as np

F32, BF16, U32 = jnp.float32, jnp.bfloat16, jnp.uint32
S, D, F = 2048, 512, 1792
WIN = 8
HALO = WIN - 1
NB = 8
LOG2E = 1.4426950408889634
EXP_SCALE = np.float32(0.25 * LOG2E)
MASKED = np.float32(-4e9)

LHS7 = ((0, 1, 3), (2, 1, 3), (0, 0, 0), (3, 0, 0), (0, 1, 1), (2, -1, 0), (1, -1, 3))
RHS7 = ((0, 1, 3), (0, 0, 0), (1, -1, 3), (2, -1, 0), (3, 0, 0), (0, 1, 1), (2, 1, 3))
STREAM = (0, 1, 2, 5, 3, 4, 6)
ROWS = (0, 3, 2, 6, 4, 5, 1)

LATENCY = 131
SLACK, ROLL_SLACK = 450, 640
NORM_PACE = {4: (18, 210), 8: (14, 190)}
NORM_TIME = 620
LEAD = 100
Q7, O7, Q49 = 2688, 3584, 2352
TILE, SEVENTH = 3136, 1600

part = functools.partial


def _pack(x):
    return pltpu.bitcast(lax.convert_element_type(x, BF16), U32)


def _unpack(x):
    return lax.convert_element_type(pltpu.bitcast(x, BF16), F32)


def _cut(x, r0, nr, c0=0, nc=None):
    nc = x.shape[1] if nc is None else nc
    return x if (nr, nc) == x.shape else lax.slice(x, (r0, c0), (r0 + nr, c0 + nc))


def _join(xs, axis):
    return xs[0] if len(xs) == 1 else lax.concatenate(xs, axis)


def _tile(x, shape):
    return _join([_join([x] * (shape[1] // x.shape[1]), 1)] * (shape[0] // x.shape[0]), 0)


def _or_all(x):
    x = x if x.dtype == U32 else pltpu.bitcast(x, U32)
    return functools.reduce(lax.bitwise_or, [
        _cut(x, r, 8, c, 128) for r in range(0, x.shape[0], 8) for c in range(0, x.shape[1], 128)])


def _row_sum(x):
    return lax.broadcast_in_dim(jnp.sum(x, axis=1), (x.shape[0], 128), (0,))


def _mix(recipe, block, gate=None):
    i, sign, j = recipe
    a = block(i) if gate is None else gate(block(i))
    return a if sign == 0 else lax.add(a, block(j)) if sign > 0 else lax.sub(a, block(j))


def _mix7(recipes, blocks):
    return [_mix(r, blocks.__getitem__) for r in recipes]


def _add(a, b):
    return [lax.add(x, y) for x, y in zip(a, b)]


def _sub(a, b):
    return [lax.sub(x, y) for x, y in zip(a, b)]


def _out4(prod, order, emit=None):
    out = [None] * 4

    def done(i, v):
        out[i] = v
        if emit is not None:
            emit(i, v)

    if order == STREAM:
        m1, m2, m3 = prod(0), prod(1), prod(2)
        done(3, _add(_sub(_add(prod(5), m1), m2), m3))
        m4 = prod(3)
        done(2, _add(m2, m4))
        t = _add(m1, m4)
        m5 = prod(4)
        done(1, _add(m3, m5))
        t = _sub(t, m5)
        done(0, _add(t, prod(6)))
    elif order == ROWS:
        m1, m4, m3 = prod(0), prod(3), prod(2)
        t = _add(_add(prod(6), m1), m4)
        m5 = prod(4)
        done(0, _sub(t, m5))
        done(1, _add(m3, m5))
        t = _add(_add(prod(5), m1), m3)
        m2 = prod(1)
        done(2, _add(m2, m4))
        done(3, _sub(t, m2))
    else:
        m1 = prod(0) if order >= 1 else None
        u = _add(prod(5), m1) if order >= 2 else m1
        t = _add(prod(6), m1) if order >= 3 else m1
        m2, m4, m3, m5 = prod(1), prod(3), prod(2), prod(4)
        done(2, _add(m2, m4))
        done(1, _add(m3, m5))
        if order == 0:
            t, u = _sub(m4, m5), _sub(m3, m2)
            m1 = prod(0)
            t, u = _add(t, m1), _add(u, m1)
        else:
            t, u = _add(t, _sub(m4, m5)), _add(u, _sub(m3, m2))
        done(3, u if order >= 2 else _add(u, prod(5)))
        done(0, t if order >= 3 else _add(t, prod(6)))
    return out


class _Bank:
    def __init__(self, ref, rows, cols):
        self.ref, self.rows, self.cols = ref, rows, cols
        self.per_row = ref.shape[1] // cols
        self.filled = {}

    def _index(self, n, r0, nr, c0, nc):
        r = (n // self.per_row) * self.rows + r0
        c = (n % self.per_row) * self.cols + c0
        return slice(r, r + nr), slice(c, c + nc)

    def put(self, n, r0, c0, x):
        idx = self._index(n, r0, x.shape[0] // 2, c0, x.shape[1])
        self.ref[idx] = _pack(x)
        for c in range(c0, c0 + x.shape[1], 128):
            for r in range(r0, r0 + x.shape[0] // 2, 8):
                key = n + c // self.cols, r
                self.filled[key] = self.filled.get(key, 0) + 128
        return idx

    def get(self, n, r0=0, nr=None):
        nr = self.rows if nr is None else nr
        if any(self.filled.get((n, r), 0) != self.cols for r in range(r0, r0 + nr, 8)):
            return None
        return self.ref[self._index(n, r0, nr, 0, self.cols)]


class _Clock:
    def __init__(self, sample):
        self.flag = jnp.where(jnp.abs(sample) < 0.0, 1, 0)
        self.masks = {}
        self.free = [0] * 4
        self.recent = [[] for _ in range(4)]
        self.begin = self.dots = self.count = 0
        self.now = self.follow = None
        self.tasks, self.ties, self.times, self.results = [], [], [], []
        self.tokens, self.syncs = {}, {}

    def spawn(self, task, at):
        self.count += 1
        heapq.heappush(self.tasks, (at, self.count, task))

    def pace(self, tasks, first, last, quiet=None):
        base = sum(self.free) / 4
        spans = [(first, last)]
        if quiet is not None:
            period, a, b = quiet
            spans = [(max(n * period + a, first), min(n * period + b, last))
                     for n in range(int(last // period) + 1)]
            spans = [(a, b) for a, b in spans if a < b]
        total = sum(b - a for a, b in spans)
        for i, task in enumerate(tasks):
            t = total * i / max(len(tasks) - 1, 1)
            for a, b in spans:
                if t <= b - a:
                    break
                t -= b - a
            self.spawn(task, base + min(a + t, b))

    def run(self, until=float("inf")):
        while self.tasks and self.tasks[0][0] <= until:
            self.now, _, task = heapq.heappop(self.tasks)
            sleep = next(task, None)
            if sleep is not None:
                self.spawn(task, self.now + sleep)
        self.now = None

    def result(self, at):
        i = bisect.bisect_right(self.times, at)
        if i == 0:
            return None
        n, m, r = self.results[i - 1]
        if (n, r) not in self.tokens:
            self.tokens[n, r] = _cut(m, r, 8, 0, 128)
        return self.tokens[n, r]

    def select(self, reg, x):
        if x.shape not in self.masks:
            self.masks[x.shape] = _tile(self.flag, x.shape) != 0
        reg = reg if reg.dtype == x.dtype else pltpu.bitcast(reg, x.dtype)
        return lax.select(self.masks[x.shape], _tile(reg, x.shape), x)

    def gate(self, x):
        token = self.result(self.now)
        if token is None:
            return x
        return self.select(token if self.follow is None else self.follow, x)

    def tie(self, x, after):
        self.ties.append((self.now + after, _or_all(x)))

    def zero(self, reg):
        return self.select(reg, self.flag)[0, 0]

    def lockstep(self, at):
        if at not in self.syncs:
            picks = {}
            for recent in self.recent:
                for begin, n, m, col in reversed(recent):
                    r = min((at - 10 - LATENCY - begin) // 8 * 8, m.shape[0] - 8)
                    if r >= 0:
                        picks[n, r, col] = m
                        break
            regs = [_cut(m, r, 8, col, 128) for (_, r, col), m in picks.items()]
            self.syncs[at] = _or_all(_join(regs, 0)) if regs else None
        return self.syncs[at]

    def fetch(self, get):
        while (x := get()) is None:
            self.run(self.tasks[0][0])
        return x

    def dot(self, lhs, rhs, nt=False):
        self.run(max(self.times[-1:] + [min(self.free)]))
        lhs, rhs = self.fetch(lhs), self.fetch(rhs)
        rhs = rhs if rhs.dtype == BF16 else pltpu.bitcast(rhs, BF16)
        nreg, kt = lhs.shape[0] // 8, lhs.shape[1] // 128
        units, starts = [], []
        for _ in range(kt * (rhs.shape[0 if nt else 1] // 128)):
            units.append(min(range(4), key=self.free.__getitem__))
            starts.append(self.free[units[-1]])
            self.free[units[-1]] += 16 * nreg
        self.begin = max(starts)
        ties, later = {}, []
        for t, x in self.ties:
            reg = max(int((t - self.begin) // 16), 0)
            if reg >= nreg:
                later.append((t, x))
            else:
                ties[reg] = x if reg not in ties else lax.bitwise_or(ties[reg], x)
        self.ties = later
        sync = self.lockstep(min(starts))
        if sync is not None:
            ties[0] = sync if 0 not in ties else lax.bitwise_or(ties[0], sync)
        parts, r = [], 0
        for reg in sorted(ties):
            if 8 * reg > r:
                parts.append(_cut(lhs, r, 8 * reg - r))
            if reg == 0 or kt == 1:
                parts.append(self.select(ties[reg], _cut(lhs, 8 * reg, 8)))
            else:
                parts.append(_join([self.select(ties[reg], _cut(lhs, 8 * reg, 8, 0, 128)),
                                    _cut(lhs, 8 * reg, 8, 128, 128 * (kt - 1))], 1))
            r = 8 * reg + 8
        if r < lhs.shape[0]:
            parts.append(_cut(lhs, r, lhs.shape[0] - r))
        dims = (((1,), (1 if nt else 0,)), ((), ()))
        m = lax.dot_general(pltpu.bitcast(_join(parts, 0), BF16), rhs, dims, preferred_element_type=F32)
        for n, i in enumerate(units):
            self.recent[i] = self.recent[i][-2:] + [(starts[n], self.dots, m, 128 * (n // kt))]
        for r in range(0, 16 * nreg, 8):
            i = bisect.bisect_right(self.times, starts[0] + LATENCY + r)
            self.times.insert(i, starts[0] + LATENCY + r)
            self.results.insert(i, (self.dots, m, r))
        self.dots += 1
        return m

    def out16(self, prod, order, emit=None):
        def outer(p):
            return [b[0] for b in _out4(lambda q: [prod(7 * p + q)], self.free.count(min(self.free)) % 4)]

        def leave(i, v):
            for j in (2, 1, 3, 0):
                emit(2 * (i // 2) + j // 2, 2 * (i % 2) + j % 2, v[j])

        return _out4(outer, order, None if emit is None else leave)


def _kernel(x_hbm, wqkv_hbm, wo_hbm, wg_hbm, wu_hbm, wd_hbm, out_hbm,
            x_in, wqkv_in, wo_in, wg_in, wu_in, wd_in, out_st,
            x_w, wo_w, out_w, pack_r, xs, qs, ks, vs, heads,
            perm_r, wqt_r, xb7_r, wq7_r, oa7_r, wo7_r, xb49_r, wq49_r, oa49_r, wo49_r,
            xa_r, wgu_r, ha49_r, ha7_r, wd49_r, wd7_r, sems, *, pacing):
    perm, wqt = _Bank(perm_r, 64, 128), _Bank(wqt_r, 192, 128)
    xb7, wq7 = _Bank(xb7_r, 256, 256), _Bank(wq7_r, 96, 256)
    oa7, wo7 = _Bank(oa7_r, 256, 256), _Bank(wo7_r, 128, 256)
    xb49, wq49 = _Bank(xb49_r, 64, 128), _Bank(wq49_r, 96, 128)
    oa49, wo49 = _Bank(oa49_r, 128, 128), _Bank(wo49_r, 64, 128)
    xa, wgu = _Bank(xa_r, 128, 128), _Bank(wgu_r, 64, 128)
    ha49, ha7 = _Bank(ha49_r, 128, 128), _Bank(ha7_r, 256, 128)
    wd49, wd7 = _Bank(wd49_r, 64, 128), _Bank(wd7_r, 64, 128)

    def x_part(h, s, m0=0, m=64):
        return [(x_hbm.at[pl.ds(64 * h + m0, m), pl.ds(8 * s, 8)], x_in.at[h, s, pl.ds(m0, m)])]

    def wqkv_part(g, n):
        return [(wqkv_hbm.at[:, pl.ds(c, 128 * n)], wqkv_in.at[:, pl.ds(c, 128 * n)])
                for c in range(128 * g, 3 * D, D)]

    waves = [x_part(0, 1, 0, 32), wqkv_part(0, 1), x_part(0, 1, 32, 32), wqkv_part(1, 1), x_part(0, 0),
             x_part(1, 1), wqkv_part(2, 2), x_part(1, 0),
             [(wo_hbm, wo_in), (wg_hbm, wg_in), (wu_hbm, wu_in)], [(wd_hbm, wd_in)]]

    def start(*which):
        for n in which:
            for src, dst in waves[n]:
                pltpu.make_async_copy(src, dst, sems.at[n]).start()

    def wait(n, zero=0):
        for src, dst in waves[n]:
            pltpu.make_async_copy(src, dst, sems.at[n + zero]).wait()

    def arrive(n, early=150):
        wait(n, clock.zero(clock.result(max(min(clock.free) - early, clock.times[0]))))

    start(0, 1, 2)
    row = lax.broadcasted_iota(jnp.int32, (128, 128), 0)
    col = lax.broadcasted_iota(jnp.int32, (128, 128), 1)
    perm.put(0, 0, 0, jnp.where(col == (row & 7) * 16 + (row >> 3), 1.0, 0.0))
    first_m = {n: lax.broadcasted_iota(jnp.int32, (n, 128), 1) < 2 for n in (8, 32)}
    wait(0)
    start(3, 4)
    clock = _Clock(x_in[0, 1, 0, :, :128].astype(F32))

    def put7(bank, r0, c0, values, n0=0, stride=1):
        idx = [bank.put(n0 + stride * i, r0, c0, v) for i, v in enumerate(values)]
        clock.tie(functools.reduce(lax.bitwise_or, [bank.ref[i] for i in idx]), SLACK)

    def build7(recipes, p, block, bank, n0, r0, gate=None):
        sums = [None] * 4
        for j in (0, 2, 3, 1) if recipes is LHS7 else (0, 1, 3, 2):
            sums[j] = _mix(recipes[p], lambda i: block(2 * (i // 2) + j // 2, 2 * (i % 2) + j % 2),
                           gate if recipes[p][1] or j in (0, 3) else None)
            clock.follow = _cut(sums[j], 8, 8)
        clock.follow = None
        idx = bank.put(n0 + 7 * p, r0, 0, _join(_mix7(recipes, sums), 1))
        clock.tie(bank.ref[idx], SLACK)
        yield from ()

    def layernorm(rows):
        x = [xs[pl.ds(r + i, 8), :] for r in rows for i in (0, 8)]
        step, pause = NORM_PACE[len(x)]
        mean, c, var = [], [], []
        for v in x:
            s = clock.gate(_cut(v, 0, 8, 0, 128))
            for k in (128, 256, 384):
                s = lax.add(s, _cut(v, 0, 8, k, 128))
            mean.append(lax.mul(_row_sum(s), np.float32(1 / D)))
            yield step
        yield pause - len(x) * step
        for v, m in zip(x, mean):
            c.append(lax.sub(v, _tile(m, v.shape)))
            var.append(_row_sum(lax.mul(c[-1], c[-1])))
            yield step
        yield pause - len(x) * step + 30
        scale = []
        for s in var:
            s = lax.add(lax.mul(s, np.float32(1 / D)), np.float32(1e-5))
            scale.append(lax.exp2(lax.mul(lax.log(s), np.float32(-0.5 * LOG2E))))
        return [(_join(c[i:i + 2], 0), _join(scale[i:i + 2], 0)) for i in range(0, len(x), 2)]

    def norm49(pieces, recipes, bank, order):
        done = {}

        def norm(i, rows):
            xn = yield from layernorm(rows)
            clock.tie(_join([s for _, s in xn], 0), SLACK)
            done[i] = [([_cut(v, 0, 16, 128 * k, 128) for k in range(4)], s) for v, s in xn]

        def step(p, i, n0, r0):
            while i not in done:
                yield 24
            scale = functools.cache(lambda n: clock.gate(done[i][n][1]))

            def block(r, c):
                n, k = (r, c) if recipes is LHS7 else (c, r)
                return lax.mul(done[i][n][0][k], scale(n))
            yield from build7(recipes, p, block, bank, n0, r0)

        return ([norm(i, rows) for i, (rows, _, _) in enumerate(pieces)],
                [step(p, i, n0, r0) for p in order for i, (_, n0, r0) in enumerate(pieces)])

    def prep_qkv7(g):
        w = _join([clock.dot(part(perm.get, 0), lambda: wqkv_in[:, c0:c0 + 128], nt=True)
                   for c0 in range(128 * g, 3 * D, D)], 0)
        wqt.put(4 * g, 0, 0, w)
        for p, v in enumerate(_mix7(LHS7, [_cut(w, r, 192, c, 256) for r in (0, 192) for c in (0, 256)])):
            wq7.put(7 * g + p, 0, 0, v)

    @functools.cache
    def words(name, r, c):
        if name == "qkv":
            return clock.fetch(part(wqt.get, c, r, 8))
        if name == "out":
            return wo_w[c, pl.ds(r, 8, stride=8), :]
        return pltpu.bitcast(dict(gate=wg_in, up=wu_in, down=wd_in)[name][r:r + 16, c:c + 128], U32)

    def slab(name, r, c):
        return _unpack(clock.gate(words(name, r, c)))

    def prep_qkv49(r):
        def block(u, b, k):
            return slab("qkv", 96 * (b % 2) + 8 * u, 4 * (2 * r + b // 2) + k)
        return [build7(LHS7, p, part(block, u), wq49, 49 * r, 8 * u) for p in STREAM for u in range(12)]

    def wo_rows(dd, g, t):
        w = clock.gate(words("out", 64 * g + dd, t))
        return _join([pltpu.bitcast(lax.shift_left(w, np.uint32(16)), F32),
                      pltpu.bitcast(lax.bitwise_and(w, np.uint32(0xFFFF0000)), F32)], 0)

    def prep_wo7():
        def step(gi, ti, dd):
            put7(wo7, 64 * gi + 8 * dd, 128 * ti,
                 _mix7(RHS7, [wo_rows(dd, g, t) for g in (gi, 2 + gi) for t in (ti, 2 + ti)]))
            yield from ()
        return [step(gi, ti, dd) for gi in range(2) for ti in range(2) for dd in range(8)]

    def prep_wo49():
        return [build7(RHS7, p, part(wo_rows, dd), wo49, 0, 8 * dd) for p in STREAM for dd in range(8)]

    def prep_gate_up(j):
        def block(u, k, n):
            return slab(("gate", "up")[n // 2], 128 * k + 16 * u, 896 * (n % 2) + 128 * j)
        return [build7(RHS7, p, part(block, u), wgu, 49 * j, 8 * u) for p in ROWS for u in range(8)]

    def prep_down():
        def block(jj, u, k, n):
            return slab("down", 128 * (7 * (k // 2) + 2 * jj + k % 2) + 16 * u, 128 * n)

        def odd(u, ti):
            put7(wd7, 8 * u, 0, _mix7(RHS7, [slab("down", 128 * ft + 16 * u, 128 * t)
                                             for ft in (6, 13) for t in (ti, 2 + ti)]), ti, 2)
            yield from ()

        return ([odd(u, ti) for u in range(8) for ti in range(2)]
                + [build7(RHS7, p, part(block, jj, u), wd49, 49 * jj, 8 * u)
                   for p in STREAM for jj in range(3) for u in range(8)])

    def token_row(h, q, c):
        return 1024 * h + 256 * q + 32 * c

    def norm_qkv7(h, s, quarters=range(4)):
        def task(pair, q, u):
            m0 = 16 * q + 8 * u
            if pair % 2 == 0:
                for t in range(4):
                    x_w[h, s, t, 4 * m0:4 * m0 + 32, :] = pltpu.bitcast(
                        x_in[h, s, m0:m0 + 8, :, 128 * t:128 * t + 128].reshape(64, 128), U32)
            rows = [token_row(h, q, 2 * pair + n) + 16 * u for n in range(2)]
            for n in range(2):
                xs[pl.ds(rows[n], 16), :] = _unpack(clock.gate(_join(
                    [x_w[h, s, t, pl.ds(4 * m0 + 2 * (pair % 2) + n, 8, stride=4), :] for t in range(4)], 1)))
            xn = yield from layernorm(rows)
            xn = [lax.mul(v, _tile(scale, v.shape)) for v, scale in xn]
            yield 4 * NORM_PACE[4][0]
            for c in (0, 128):
                blocks = [_cut(xn[i % 2], 0, 16, 256 * (i // 2) + c, 128) for i in range(4)]
                if c:
                    blocks[0], blocks[3] = clock.gate(blocks[0]), clock.gate(blocks[3])
                put7(xb7, 64 * pair + m0, c, _mix7(RHS7, blocks), 7 * h)
                yield 20
        return [task(pair, q, u) for q in quarters for u in range(2) for pair in (2 * s, 2 * s + 1)]

    def norm_qkv49(h, s):
        return norm49([([token_row(h, q, 4 * s + n) + 16 * u for n in range(4)], 49 * (2 * h + s), 16 * q + 8 * u)
                       for q in range(4) for u in range(2)], RHS7, xb49, STREAM)

    written = {}

    def note(*key):
        written[key] = written.get(key, 0) + 1

    def own(c):
        return slice(128 * (HALO + c), 128 * (HALO + c + 1))

    def wrap(name, h, g, c):
        ref = dict(k=ks, v=vs)[name]
        assert h == 0 or written[name, 0, g, c - NB] == written.get((name, h, g, c - NB), 0) + 1
        for r in range(0, 128, 32):
            x = pltpu.roll(ref[h, g, r:r + 32, own(c)], 2, 1)
            if h > 0:
                x = lax.select(first_m[32], ref[h - 1, g, r:r + 32, own(c - NB)], x)
            ref[h, g, r:r + 32, own(c - NB)] = x
            clock.tie(x, ROLL_SLACK)
            yield 24
        note(name, h, g, c - NB)

    def keep_qkv(h, g, c, half, x, delay):
        if half == 0:
            qs[h, g, :, 128 * c:128 * c + 128] = _cut(x, 0, 128)
            ks[h, g, :64, own(c)] = _cut(x, 128, 64)
        else:
            ks[h, g, 64:, own(c)] = _cut(x, 0, 64)
            vs[h, g, :, own(c)] = _cut(x, 64, 128)
        note("qv"[half], h, g, c)
        at = clock.begin + LATENCY + 140 + delay
        if c > 0 and half == 1:
            clock.spawn(wrap("v", h, g, c), at)
        if written.get(("q", h, g, c)) == written.get(("v", h, g, c)):
            note("k", h, g, c)
            if c > 0:
                clock.spawn(wrap("k", h, g, c), at + 64 * half)

    def qkv7(h, g, sets=(1, 0)):
        for s in sets:
            def emit(i, v):
                for n in range(2):
                    keep_qkv(h, g, 4 * s + 2 * n + i % 2, i // 2, _cut(v[0], 0, 192, 128 * n, 128), 96 * (1 - n))
            _out4(lambda p: [clock.dot(part(wq7.get, 7 * g + p), part(xb7.get, 7 * h + p, 128 * s, 128), nt=True)],
                  STREAM, emit)

    def qkv49(h, s):
        for r in range(2):
            clock.out16(
                lambda p: clock.dot(part(wq49.get, 49 * r + p), part(xb49.get, 49 * (2 * h + s) + p), nt=True),
                STREAM,
                lambda b, n, x: keep_qkv(h, 2 * r + b // 2, 4 * s + n, b % 2, x, 90 * (2 * (b % 2) + n % 2)))

    def attend_time(layer, pace):
        return 32 * pace["step"] + pace["gap"] + pace["turn"] + (0 if layer else 180 + SLACK)

    def attend(layer, h, g, c, pace):
        while any(written.get((name, h, g, n)) != layer + 1 for name in "kv" for n in range(c + 1 - NB, 4)):
            yield 24
        assert all(written[name, h, g, n] == layer + 1 for name in "kv" for n in range(c + 1))
        for d in range(16):
            q = clock.gate(qs[h, g, 8 * d:8 * d + 8, 128 * c:128 * c + 128])
            t = lax.mul(_tile(q, (8, 128 * WIN)), ks[h, g, 8 * d:8 * d + 8, 128 * c:128 * (c + WIN)])
            logit = t if d == 0 else lax.add(logit, t)
            yield pace["step"]
        logit = [_cut(logit, 0, 8, 128 * (HALO - w), 128) for w in range(WIN)]
        if h == 0:
            for w in range(c + 1, WIN):
                logit[w] = lax.select(first_m[8], lax.full((8, 128), MASKED, F32), logit[w])
        top = functools.reduce(lax.max, logit)
        e = [lax.exp2(lax.mul(lax.sub(x, top), EXP_SCALE)) for x in logit]
        inv = lax.div(lax.full((8, 128), 1, F32), functools.reduce(lax.add, e))
        prob = [lax.mul(x, inv) for x in e]
        yield pace["gap"]
        for w in range(WIN):
            t = lax.mul(_tile(clock.gate(prob[w]), (128, 128)), vs[h, g, :, own(c - w)])
            o = t if w == 0 else lax.add(o, t)
            yield 2 * pace["step"]
        o = lax.transpose(o, (1, 0))
        heads[h, g, c] = o
        note("o", h, g, c)
        clock.tie(_cut(o, 120, 8), pace["turn"])
        if layer == 0:
            yield pace["turn"]
            while any(("o", h, i, n) not in written for i in (g, g % 2) for n in (c, c | 1)):
                yield 24
            for p in (((2, 5), ()), ((0, 4, 6), (1, 3)))[g // 2][c % 2]:
                for r in (0, 64):
                    v = _mix(LHS7[p], lambda i: heads[h, g % 2 + 2 * (i % 2), c // 2 * 2 + i // 2, r:r + 64],
                             clock.gate)
                    put7(oa7, 64 * (c // 2) + r // 2, 128 * (g % 2), [v], 7 * h + p)
                    yield 30

    def heads49(h, s):
        block = functools.cache(lambda r, n, g: heads[h, g, 4 * s + n, r:r + 16])

        def step(p, r):
            while any(written["o", h, g, 4 * s + n] != 2 for g in range(2 if p in (2, 5) else 4) for n in range(4)):
                yield 24
            yield from build7(LHS7, p, part(block, r), oa49, 0, 64 * s + r // 2, clock.gate)
        return [step(p, r) for p in STREAM for r in range(0, 128, 16)]

    def add_tokens(h, c, cols, x, r0):
        for q in range(4):
            r = pl.ds(token_row(h, q, c), 32)
            xs[r, cols] = lax.add(xs[r, cols], _cut(x, r0 + 32 * q, 32))

    def out_proj7(h, s):
        def emit(i, v):
            for n in range(2):
                add_tokens(h, 4 * s + 2 * n + i // 2, pl.ds(256 * (i % 2), 256), v[0], 128 * n)
        _out4(lambda p: [clock.dot(part(oa7.get, 7 * h + p, 128 * s, 128), part(wo7.get, p))], STREAM, emit)

    def out_proj49(h, s):
        clock.out16(lambda p: clock.dot(part(oa49.get, p, 64 * s, 64), part(wo49.get, p)), STREAM,
                    lambda n, t, x: add_tokens(h, 4 * s + n, pl.ds(128 * t, 128), x, 0))
        oa49.filled.clear()

    def norm_ffn(h, sets):
        return norm49([([token_row(h, q, 0) + 16 * u for q in range(4)], 49 * h, 8 * u)
                       for u in reversed(range(16)) if u // 8 in sets], LHS7, xa, ROWS)

    hidden = {}

    def gate_up(h, sets, pace, tiles=range(7)):
        r0, n = 128 * sets[0], 128 * len(sets)

        def odd(a, p, ri, r):
            v = _mix(LHS7[p], lambda i: _cut(a[2 * (i // 2) + ri][i % 2], r, 64), clock.gate)
            put7(ha7, 128 * ri + r // 2, 0, [v], p)
            yield from ()

        for j in tiles:
            g1, u1, g2, u2 = clock.out16(
                lambda p: clock.dot(part(xa.get, 49 * h + p, r0 // 2, n // 2), part(wgu.get, 49 * j + p)), ROWS)
            hid = [lax.mul(lax.max(g, np.float32(0)), u) for g, u in zip(g1 + g2, u1 + u2)]
            hidden[j] = [hid[2 * q:2 * q + 2] for q in range(4)]
            if j == 6:
                for key in [k for k in xa.filled if k[0] // 49 == h and r0 <= 2 * k[1] < r0 + n]:
                    del xa.filled[key]
                clock.pace([odd(hidden[6], p, ri, r) for p in STREAM for ri in range(2) for r in range(0, n, 64)],
                           LATENCY + 200, pace["odd"] * n / 256)
            elif j % 2:
                block = functools.cache(
                    lambda r, q, k, pair=(hidden[j - 1], hidden[j]): _cut(pair[k % 2][q][k // 2], r, 16))
                steps = {(p, r): build7(LHS7, p, part(block, r), ha49, 49 * (j // 2), r // 2, clock.gate)
                         for r in range(0, n, 16) for p in range(7)}
                if j < 5:
                    clock.pace(list(steps.values()), *(f * n for f in pace["pairs"]))
                else:
                    clock.pace([steps[p, r] for p in STREAM for r in range(0, n, 16)],
                               LATENCY + 200, pace["pair"] * n / 256)

    sent, early, later = [], {}, []

    def finish(h, s, q, t, y, step):
        gate = clock.gate if step else lambda x: x
        cols = slice(128 * t, 128 * t + 256)
        for c in range(4):
            pack_r[16 * c:16 * c + 16, cols] = _pack(gate(_cut(y, 32 * c, 32)))
            for n in (t, t + 1):
                out_w[h, s, n, pl.ds(64 * q + c, 16, stride=4), :] = pack_r[
                    16 * c:16 * c + 16, 128 * n:128 * n + 128]
            yield step
        for r in range(64 * q, 64 * q + 64, 16):
            rows = gate(_join([out_w[h, s, n, r:r + 16, :] for n in (t, t + 1)], 1))
            out_st[h, s, r // 4:r // 4 + 4, :, cols] = pltpu.bitcast(rows, BF16).reshape(4, 8, 256)
            yield step
        note("y", h, s, q, t)

    def send(h, s, q0=0, nq=4, t0=0, nt=4):
        clock.fetch(lambda: all(("y", h, s, q, t) in written
                                for q in range(q0, q0 + nq) for t in range(t0, t0 + nt, 2)) or None)
        cols = pl.ds(128 * t0, 128 * nt)
        sent.append(pltpu.make_async_copy(
            out_st.at[h, s, pl.ds(16 * q0, 16 * nq), :, cols],
            out_hbm.at[pl.ds(64 * h + 16 * q0, 16 * nq), pl.ds(8 * s, 8), cols], sems.at[len(waves)]))
        sent[-1].start()

    def down(layer, h, sets, only=None):
        n = 128 * len(sets)
        final = (layer, h, sets) == (1, 1, (0,))

        def outer(p):
            def inner(q):
                return [functools.reduce(lax.add, [
                    clock.dot(part(ha49.get, 49 * jj + 7 * p + q, 0, n // 2), part(wd49.get, 49 * jj + 7 * p + q))
                    for jj in range(3)])]

            def odd():
                return [clock.dot(part(ha7.get, p, 128 * ri, n // 2), part(wd7.get, 2 * p + ci))
                        for ri in range(2) for ci in range(2)]

            if p == 6:
                e = odd()
                if final:
                    send(h, 0, 0, 2, 2, 2)
                    send(h, 0, 2, 2)
                return _add(e, [b[0] for b in _out4(inner, STREAM)])
            return _add([b[0] for b in _out4(inner, STREAM)], odd())

        def emit(i, v):
            for j in (2, 0):
                q, t = 2 * (i // 2) + j // 2, 2 * (i % 2)
                idx = (pl.ds(token_row(h, q, 4 * sets[0]), n), pl.ds(128 * t, 256))
                y = lax.add(xs[idx], _join(v[j:j + 2], 1))
                if final:
                    step = 50 if i >= 2 else 0
                    clock.spawn(finish(h, 0, q, t, y, step), clock.begin + LATENCY + n + 4 * step * j)
                elif layer:
                    later.append(finish(h, sets[0], q, t, y, 50))
                else:
                    xs[idx] = y

        if only is not None:
            early.update({p: outer(p) for p in only})
        else:
            _out4(lambda p: early.pop(p) if p in early else outer(p), STREAM, emit)
            ha49.filled.clear()
            ha7.filled.clear()

    def pace_norm_ffn(h, s, length, pace):
        norms, steps = norm_ffn(h, (s,))
        clock.pace(norms, LEAD, pace["split"] * length - NORM_TIME)
        clock.pace(steps, pace["split"] * length, length + pace["over"])

    def write_back(pace):
        clock.pace(list(later), *pace["store"])
        later.clear()

    def ffn_under(here, after, project, pace):
        (layer, h, s), (layer2, h2, s2) = here, after
        tiles, seventh = 3.5 * TILE, SEVENTH / 2
        cut, ahead, n = min(pace["cut"], pace["ahead"]), pace["ahead"], pace["first"]
        span = tiles + 2 * Q49 * min(len(project), 1) + seventh * ahead
        write_back(pace)
        att = [attend(layer2, h2, g, 4 * s2 + c, pace) for g in range(4) for c in reversed(range(4))]
        clock.pace(att[:n], pace["begin"], tiles - 700, pace["quiet"])
        clock.pace(att[n:], tiles, span - attend_time(layer2, pace) - layer2 * pace["end"])
        if layer2:
            clock.pace(heads49(h2, s2), span - pace["end"] + 100, span + 700)
        for i, target in enumerate(project):
            norms, steps = norm_qkv49(*target)
            first, last = ((pace["norm"], tiles + cut * seventh) if i == 0 else
                           (tiles + cut * seventh + pace["norm2"], span + O7 / 2 + (7 - ahead) * seventh))
            mid = first + pace["mid"] * (last + 600 - first)
            clock.pace(norms, first, mid - NORM_TIME)
            clock.pace(steps, mid, last + 600)
        gate_up(h, (s,), pace)
        down(layer, h, (s,), STREAM[:cut])
        for target in project[:1]:
            qkv49(*target)
        down(layer, h, (s,), STREAM[cut:ahead])
        (out_proj49 if layer2 else out_proj7)(h2, s2)
        pace_norm_ffn(h2, s2, seventh * (7 - ahead) + Q49 * len(project[1:]), pace)
        down(layer, h, (s,))
        for target in project[1:]:
            qkv49(*target)

    clock.pace(norm_qkv7(0, 1, (0, 1)), 0, 200)
    clock.run()
    wait(1, clock.zero(clock.ties[0][1]))
    clock.ties = []
    prep_qkv7(0)
    wait(2, clock.zero(_cut(clock.results[-1][1], 120, 8, 0, 128)))
    start(5)
    times, clock.times = clock.times, []
    clock.pace(norm_qkv7(0, 1, (2, 3)), 0, 200)
    clock.run()
    clock.times, clock.ties = times, []
    qkv7(0, 0, (1,))
    arrive(3)
    prep_qkv7(1)
    arrive(4, 250)
    start(6, 7)
    norm7_time = 2 * NORM_PACE[4][1] + 30 + 4 * NORM_PACE[4][0] + SLACK
    tasks = norm_qkv7(0, 0)
    clock.pace(tasks[::2], -150, Q7 / 2 - norm7_time + SLACK - 100)
    clock.pace(tasks[1::2], 200, 0.75 * Q7 - norm7_time + SLACK - 100)
    qkv7(0, 1, (1,))
    for n in range(2):
        _out4(lambda p: [clock.dot(part(wq7.get, p), part(xb7.get, p, 64 * n, 64), nt=True)], STREAM,
              lambda i, v: keep_qkv(0, 0, 2 * n + i % 2, i // 2, v[0], 48))
    arrive(5)
    pace = pacing[0]
    clock.pace([attend(0, 0, g, 4 * s + c, pace) for g, s in [(0, 1), (0, 0), (1, 1), (1, 0), (2, 1), (3, 1),
                                                              (2, 0), (3, 0)] for c in reversed(range(4))],
               pace["begin"], 768 + 5.5 * Q7 + O7 / 2 - attend_time(0, pace) + pace["end"])
    clock.pace(norm_qkv7(1, 1) + norm_qkv7(1, 0), pace["norm"], 768 + pace["norm2"] * Q7 - norm7_time)
    qkv7(0, 1, (0,))
    arrive(6)
    start(8)
    prep_qkv7(2)
    prep_qkv7(3)
    arrive(7)
    qkv7(0, 2)
    qkv7(0, 3)
    for g in range(3):
        qkv7(1, g, (1,))
    arrive(8)
    start(9)
    for t in range(4):
        wo_w[t, :256] = pltpu.bitcast(wo_in[:, 128 * t:128 * t + 128], U32)
    clock.pace(prep_wo7(), LEAD, pace["wo"] * Q7)
    clock.pace(prep_gate_up(0) + prep_gate_up(1), Q7, 1.5 * Q7 + O7 + pace["prep"])
    for g in range(3):
        qkv7(1, g, (0,))
    out_proj7(0, 1)
    norms, steps = norm_ffn(0, (0, 1))
    clock.pace(norms[:8], LEAD, O7 / 2 - 100)
    out_proj7(0, 0)
    clock.pace(norms[8:], LEAD + 100, pace["mid"] * Q7)
    clock.pace(steps, pace["split"] * Q7, Q7 + pace["over"])
    qkv7(1, 3)

    pace, pace2 = pacing[1], pacing[2]
    n1, n2 = pace["first"]
    att = [attend(0, 1, g, 4 + c, pace if g < 2 else pace2) for g in range(4) for c in reversed(range(4))]
    for j in range(2, 7):
        clock.pace(prep_gate_up(j), TILE * (j - pace["prep"]), TILE * (j + 1 - pace["prep"]) - 60)
    clock.pace(att[:n1], pace["begin"] * TILE, 2 * TILE, pace["quiet"])
    clock.pace(att[n1:n1 + n2], 2 * TILE + 300, 7 * TILE - 300, pace["quiet"])
    clock.pace(prep_down(), (7 - pace["prep"]) * TILE, 7 * TILE + pace2["prep"])
    gate_up(0, (0, 1), pace, range(5))
    arrive(9)
    gate_up(0, (0, 1), pace2, (5, 6))
    clock.pace(att[n1 + n2:], pace2["begin"], SEVENTH * pace2["ahead"] - attend_time(0, pace2))
    clock.pace(prep_qkv49(0) + prep_qkv49(1), *pace2["wq"])
    down(0, 0, (0, 1), STREAM[:pace2["ahead"]])
    out_proj7(1, 1)
    pace_norm_ffn(1, 1, SEVENTH * (7 - pace2["ahead"]), pace2)
    down(0, 0, (0, 1))

    ffn_under((0, 1, 1), (0, 1, 0), [(0, 1), (0, 0)], pacing[3])
    clock.pace(prep_wo49(), *pacing[4]["wo"])
    ffn_under((0, 1, 0), (1, 0, 1), [(1, 1)], pacing[4])
    ffn_under((1, 0, 1), (1, 0, 0), [(1, 0)], pacing[5])
    ffn_under((1, 0, 0), (1, 1, 1), [], pacing[6])
    ffn_under((1, 1, 1), (1, 1, 0), [], pacing[7])
    write_back(pacing[8])
    gate_up(1, (0,), pacing[8])
    send(0, 1)
    send(0, 0)
    send(1, 1)
    down(1, 1, (0,))
    send(1, 0, 0, 2, 0, 2)
    for copy in sent:
        copy.wait()


_COMMON = dict(step=14, gap=50, turn=420, begin=900, end=1200, first=7, cut=3, ahead=4, norm=1500,
               mid=0.5, split=0.55, over=900, odd=5000, pair=4500, pairs=(2, 26), store=(2000, 16000),
               quiet=(1568, 131, 400))
PACING = [dict(_COMMON, **stage) for stage in [
    dict(step=12, gap=40, begin=0, end=200, norm=0, norm2=4, mid=0.4, split=0.8, over=2200, wo=0.8, prep=0),
    dict(step=12, turn=350, begin=0.6, first=(2, 4), pairs=(0.5, 24.5), quiet=(3136, 130, 700), prep=1),
    dict(step=15, turn=500, begin=800, ahead=5, over=1150, odd=6500, pair=3800, prep=7584, wq=(8200, 24000)),
    dict(step=15, gap=70, turn=500, end=900, ahead=3, norm2=3500, mid=0.7, split=0.7, odd=4000, pair=5500),
    dict(gap=40, begin=1400, norm=600, split=0.85, over=600, wo=(11000, 17000)),
    dict(turn=500, cut=4, ahead=5, mid=0.6, split=0.7),
    dict(step=12, gap=70, turn=350, end=900, first=10, odd=4000, store=(10000, 17500), pairs=(2.5, 26)),
    dict(gap=40, turn=350, begin=1400, end=900, first=10, split=0.7, over=600, store=(6000, 17000),
         quiet=(1568, 100, 450)),
    dict(odd=4000, pair=5500, store=(1200, 9500)),
]]


def _forward(pacing, A_x, A_wqkv, A_wo, B_W_gate, B_W_up, B_W_down):
    vm = pltpu.VMEM
    scratch = [
        vm((2, 2, 64, 8, D), BF16),
        vm((D, 3 * D), BF16),
        vm((D, D), BF16),
        vm((D, F), BF16),
        vm((D, F), BF16),
        vm((F, D), BF16),
        vm((2, 2, 64, 8, D), BF16),
        vm((2, 2, 4, 264, 128), U32),
        vm((4, 264, 128), U32),
        vm((2, 2, 4, 264, 128), U32),
        vm((64, D), U32),
        vm((S, D), F32),
        vm((2, 4, 128, 128 * NB), F32),
        vm((2, 4, 128, 128 * (NB + HALO)), F32),
        vm((2, 4, 128, 128 * (NB + HALO)), F32),
        vm((2, 4, NB, 128, 128), F32),
        vm((64, 256), U32),
        vm((4 * 192, 512), U32),
        vm((14 * 256, 256), U32),
        vm((28 * 96, 256), U32),
        vm((14 * 256, 256), U32),
        vm((7 * 128, 256), U32),
        vm((28 * 64, 896), U32),
        vm((14 * 96, 896), U32),
        vm((7 * 128, 896), U32),
        vm((7 * 64, 896), U32),
        vm((14 * 128, 896), U32),
        vm((49 * 64, 896), U32),
        vm((21 * 128, 896), U32),
        vm((256, 896), U32),
        vm((21 * 64, 896), U32),
        vm((2 * 64, 896), U32),
        pltpu.SemaphoreType.DMA((11,)),
    ]
    in_hbm = pl.BlockSpec(memory_space=pl.ANY)
    out = pl.pallas_call(
        part(_kernel, pacing=pacing),
        out_shape=jax.ShapeDtypeStruct((S // 16, 16, D), BF16),
        in_specs=[in_hbm] * 6,
        out_specs=in_hbm,
        scratch_shapes=scratch,
        compiler_params=pltpu.CompilerParams(
            vmem_limit_bytes=110 * 2**20,
            flags={"XLA_TPU_RESCHEDULE_DMA_DONES": True}),
        name="fused",
    )(A_x.reshape(S // 16, 16, D), A_wqkv, A_wo, B_W_gate, B_W_up, B_W_down)
    return out.reshape(1, S, D)


@jax.jit
def pallas_interleave_layers__sliding_local_dilated__glu_gated_reglu__prompt_kernel(
    A_x: jax.Array,
    A_wqkv: jax.Array,
    A_wo: jax.Array,
    B_x: jax.Array,
    B_W_gate: jax.Array,
    B_W_up: jax.Array,
    B_W_down: jax.Array,
):
    del B_x
    return _forward(PACING, A_x, A_wqkv, A_wo, B_W_gate, B_W_up, B_W_down)
```
